```python
import jax
import jax.numpy as jnp

def _softmax(x, axis=-1):
    return jax.nn.softmax(x, axis=axis)
def _gelu(x):
    return jax.nn.gelu(x, approximate=True)
def _silu(x):
    return jax.nn.silu(x)
def _sigmoid(x):
    return jax.nn.sigmoid(x)
def _layernorm(x, axis=-1, eps=1e-5):
    m = jnp.mean(x, axis=axis, keepdims=True)
    v = jnp.var(x, axis=axis, keepdims=True)
    return (x - m) / jnp.sqrt(v + eps)
def _scatter_add(tgt, idx, src, axis=0):
    return tgt.at[idx].add(src)
def _segment_sum(src, seg, n):
    return jax.ops.segment_sum(src, seg, n)
class _Rng:
    def __init__(self, key):
        self._k = key
    def _next(self):
        self._k, sub = jax.random.split(self._k)
        return sub
    def normal(self, shape):
        return jax.random.normal(self._next(), shape, dtype=jnp.bfloat16)
    def randint(self, lo, hi, shape):
        return jax.random.randint(self._next(), shape, lo, hi, dtype=jnp.int32)
    def uniform(self, shape, lo=0.0, hi=1.0):
        return jax.random.uniform(self._next(), shape, jnp.bfloat16, lo, hi)
    def permutation(self, n):
        return jax.random.permutation(self._next(), n)


kernel_name = 'concat_heads__gqa_block_cached__compressed_kv_cla__decode'

def setup_inputs():
    _rng = _Rng(jax.random.key(int.from_bytes(__import__("os").urandom(4), "little")))
    _w = (lambda a: (lambda t: t.astype(jnp.bfloat16) if jnp.issubdtype(t.dtype, jnp.floating) else t)(jnp.asarray(a)))
    def _A_setup():
        B, Sq, D = 2, 1, 512
        Hq, Hkv, Sk, Dh = 32, 32, 8192, 128
        assert Hq % Hkv == 0, (Hq, Hkv)
        return {
            "x": _w((lambda *s: _rng.normal(s) * 0.05)(B, Sq, D)),
            "k_cache": _w((lambda *s: _rng.normal(s) * 0.05)(B, Hkv, Sk, Dh)),
            "v_cache": _w((lambda *s: _rng.normal(s) * 0.05)(B, Hkv, Sk, Dh)),
            "wq": _w((lambda *s: _rng.normal(s) * 0.05)(D, Hq * Dh) * (D ** -0.5)),
            "wo": _w((lambda *s: _rng.normal(s) * 0.05)(Hq * Dh, D) * ((Hq * Dh) ** -0.5)),
        }
    _A_in = _A_setup()

    def _B_setup():
        B, H, Sq, Sk, D, M = 2, 32, 1, 8192, 128, 512
        Dc = 4 * D
        return {
            "x": _w((lambda *s: _rng.normal(s) * 0.05)(B, Sq, M)),
            "c_kv": _w((lambda *s: _rng.normal(s) * 0.05)(B, Sk, Dc)),
            "w_q": _w((lambda *s: _rng.normal(s) * 0.05)(M, H, D) * (M ** -0.5)),
            "w_uk": _w((lambda *s: _rng.normal(s) * 0.05)(Dc, H, D) * (Dc ** -0.5)),
            "w_uv": _w((lambda *s: _rng.normal(s) * 0.05)(Dc, H, D) * (Dc ** -0.5)),
            "w_o": _w((lambda *s: _rng.normal(s) * 0.05)(H, D, M) * ((H * D) ** -0.5)),
        }
    _B_in = _B_setup()

    return {
        "A_x": _A_in["x"],
        "A_k_cache": _A_in["k_cache"],
        "A_v_cache": _A_in["v_cache"],
        "A_wq": _A_in["wq"],
        "A_wo": _A_in["wo"],
        "B_x": _B_in["x"],
        "B_c_kv": _B_in["c_kv"],
        "B_w_q": _B_in["w_q"],
        "B_w_uk": _B_in["w_uk"],
        "B_w_uv": _B_in["w_uv"],
        "B_w_o": _B_in["w_o"],
    }

def reference(A_x, A_k_cache, A_v_cache, A_wq, A_wo, B_x, B_c_kv, B_w_q, B_w_uk, B_w_uv, B_w_o):
    def _A_ref(x, k_cache, v_cache, wq, wo):
        B, Sq, D = x.shape
        Hq, Dh = 32, 128
        Hkv = k_cache.shape[1]
        rep = Hq // Hkv
        q = (lambda x, *d: x.transpose(*d))((x @ wq).reshape(B, Sq, Hq, Dh), 0, 2, 1, 3)
        k = jnp.repeat(k_cache, rep, axis=1)
        v = jnp.repeat(v_cache, rep, axis=1)
        scores = jnp.einsum("bhqd,bhkd->bhqk", q, k) * (Dh ** -0.5)
        p = _softmax(scores, axis=-1)
        o = jnp.einsum("bhqk,bhkd->bhqd", p, v)
        return (lambda x, *d: x.transpose(*d))(o, 0, 2, 1, 3).reshape(B, Sq, Hq * Dh) @ wo

    def _B_ref(x, c_kv, w_q, w_uk, w_uv, w_o):
        B, Sq, M = x.shape[0], x.shape[1], x.shape[2]
        Sk = c_kv.shape[1]
        H, D = w_q.shape[1], w_q.shape[2]
        q = jnp.einsum("bqm,mhd->bhqd", x, w_q)
        k = jnp.einsum("bkc,chd->bhkd", c_kv, w_uk)
        v = jnp.einsum("bkc,chd->bhkd", c_kv, w_uv)
        scores = jnp.einsum("bhqd,bhkd->bhqk", q, k) * (D ** -0.5)
        off = Sk - Sq
        qi = jnp.arange(Sq)[:, None]
        kj = jnp.arange(Sk)[None, :]
        cmask = kj <= (qi + off)
        scores = jnp.where(cmask[None, None], scores, -1e9)
        p = _softmax(scores, axis=-1)
        ctx = jnp.einsum("bhqk,bhkd->bhqd", p, v)
        return jnp.einsum("bhqd,hdm->bqm", ctx, w_o)

    a = _A_ref(A_x, A_k_cache, A_v_cache, A_wq, A_wo)
    b = _B_ref(B_x, B_c_kv, B_w_q, B_w_uk, B_w_uv, B_w_o)
    return jnp.concatenate([a, b], axis=-1)
```

```python
import functools
import jax
import jax.numpy as jnp
from jax.experimental import pallas as pl
from jax.experimental.pallas import tpu as pltpu

F32, BF16 = jnp.float32, jnp.bfloat16
NB, NH, S, DH, DM, DC = 2, 32, 8192, 128, 512, 512
NHEAD = NB * NH


def _pieces(total, step):
    out, o = [], 0
    while o < total:
        r = min(step, total - o)
        out.append((o, r))
        o += r
    return out


def make_kernel(dis=(), kv_rows=192, slabs=6, ckv_rows=48, bchunk=2048,
                i_wu=0, i_ckv=2, i_qb=0, i_qabs=3, i_b=12, i_ctx=21,
                wo_chunks=((0, 16), (16, 8), (24, 8)), unroll=8, nbc=False, cpc=64, R=3, piece_first=False):
    kv_pieces = _pieces(S, kv_rows)
    nch = len(wo_chunks)
    nbj = S // bchunk
    ncp = DC // cpc
    SEM_AX, SEM_BX, SEM_X, SEM_WQ, SEM_WQB, SEM_WUK, SEM_WUV = range(7)
    SEM_CKV = 7
    SEM_WO = SEM_CKV + nbj
    SEM_K = SEM_WO + 2 * nch
    SEM_V = SEM_K + R
    NSEM = SEM_V + R
    LA = R - 1

    def kernel(ax_hbm, bx_hbm, k_hbm, v_hbm, wq_hbm, wo_hbm, ckv_hbm, wqb_hbm, wuk_hbm, wuv_hbm, wob_hbm,
               o_ref,
               kbuf, vbuf, wq_v, wqb_v, wuk_v, wuv_v, ckv_v, wo_v, wob_v,
               ax_v, bx_v, xb_v, xb_s, qa_scr, oa_scr, qb_scr, qabs_scr, m_scr, l_scr, pc_scr, ctx_scr, sems):

        def copy(src, dst, sem):
            return pltpu.make_async_copy(src, dst, sems.at[sem])

        def wait_all(buf, sem):
            pltpu.make_async_copy(buf, buf, sems.at[sem]).wait()

        def start_head(i, slot):
            b = i // NH
            h = i % NH
            for (o, r) in kv_pieces:
                copy(k_hbm.at[b, h, pl.ds(o, r)], kbuf.at[slot, pl.ds(o, r)], SEM_K + slot).start(priority=0)
                copy(v_hbm.at[b, h, pl.ds(o, r)], vbuf.at[slot, pl.ds(o, r)], SEM_V + slot).start(priority=1)

        def start_wq_pair():
            a = [(r, c, n) for r in range(0, DM, 16) for (c, n) in ((0, 1536), (1536, 1536), (3072, 1024))]
            bp = _pieces(DM, slabs)
            for t in range(max(len(a), len(bp))):
                if t < len(a):
                    r, c, n = a[t]
                    copy(wq_hbm.at[pl.ds(r, 16), pl.ds(c, n)], wq_v.at[pl.ds(r, 16), pl.ds(c, n)], SEM_WQ).start(priority=0)
                if t < len(bp):
                    o, n = bp[t]
                    copy(wqb_hbm.at[pl.ds(o, n)], wqb_v.at[pl.ds(o, n)], SEM_WQB).start(priority=1)

        def start_wu(half):
            pcs = _pieces(DM, slabs)
            hh = (len(pcs) + 1) // 2
            for (o, n) in (pcs[:hh] if half == 0 else pcs[hh:]):
                copy(wuk_hbm.at[pl.ds(o, n)], wuk_v.at[pl.ds(o, n)], SEM_WUK).start(priority=0)
                copy(wuv_hbm.at[pl.ds(o, n)], wuv_v.at[pl.ds(o, n)], SEM_WUV).start(priority=1)

        def start_ckv(j):
            base = pl.multiple_of(j * bchunk, bchunk)
            for (o, r) in _pieces(bchunk, ckv_rows):
                copy(ckv_hbm.at[0, pl.ds(base + o, r)], ckv_v.at[0, pl.ds(base + o, r)], SEM_CKV + j).start(priority=0)
                copy(ckv_hbm.at[1, pl.ds(base + o, r)], ckv_v.at[1, pl.ds(base + o, r)], SEM_CKV + j).start(priority=1)

        def start_wo(ci):
            h0, nh = wo_chunks[ci]
            for h in range(h0, h0 + nh):
                for (o, r) in _pieces(128, ckv_rows):
                    copy(wo_hbm.at[pl.ds(h * 128 + o, r)], wo_v.at[pl.ds(h * 128 + o, r)], SEM_WO + ci).start(priority=0)
                    copy(wob_hbm.at[h, pl.ds(o, r)], wob_v.at[h, pl.ds(o, r)], SEM_WO + nch + ci).start(priority=1)

        ax_copy = copy(ax_hbm, ax_v, SEM_AX)
        bx_copy = copy(bx_hbm, bx_v, SEM_BX)
        ax_copy.start(priority=0)
        bx_copy.start(priority=1)
        start_wq_pair()
        for i0 in range(LA):
            start_head(i0, i0)

        ax_copy.wait()
        bx_copy.wait()
        axf = ax_v[...].astype(F32)
        xa = jnp.concatenate([jnp.broadcast_to(axf[b:b + 1, :], (8, DM)) for b in range(NB)], axis=0).astype(BF16)
        xb_v[...] = jnp.concatenate([bx_v[...].astype(F32), jnp.zeros((8 - NB, DM), F32)], axis=0)
        xcopy = copy(xb_v, xb_s, SEM_X)
        xcopy.start()

        z = jnp.zeros((NH, DH), F32)
        for b in range(NB):
            qb_scr[b] = z
            ctx_scr[b] = z
            m_scr[b] = jnp.full((NH, DH), -jnp.inf, F32)
            l_scr[b] = z
            for cc in range(DC // 128):
                pc_scr[b, cc] = z
                qabs_scr[b, cc] = z

        wait_all(wq_v, SEM_WQ)
        qa = jnp.dot(xa, wq_v[...], preferred_element_type=F32)
        for b in range(NB):
            for h in range(NH):
                qa_scr[b * NH + h] = qa[b * 8:(b + 1) * 8, h * DH:(h + 1) * DH]

        lane = jax.lax.broadcasted_iota(jnp.int32, (NH, DH), 1)

        def phase_qb(part):
            @pl.when(part == 0)
            def _():
                xcopy.wait()
                wait_all(wqb_v, SEM_WQB)
            if "qb" in dis:
                return
            m0 = part * (DM // 2)

            def body(t, accs):
                m = m0 + t
                w = wqb_v[m].astype(F32)
                return tuple(accs[b] + w * xb_s[b, m] for b in range(NB))
            accs = jax.lax.fori_loop(0, DM // 2, body, tuple(qb_scr[b] for b in range(NB)), unroll=unroll)
            for b in range(NB):
                qb_scr[b] = accs[b]

        def phase_qabs(t):
            cc = t // (128 // cpc)
            j0 = (t % (128 // cpc)) * cpc

            @pl.when(t == 0)
            def _():
                wait_all(wuk_v, SEM_WUK)
            q = [qb_scr[b] for b in range(NB)]

            def body(jj, accs):
                j = j0 + jj
                w = wuk_v[cc * 128 + j].astype(F32)
                out = []
                for b in range(NB):
                    r = jnp.sum(w * q[b], axis=1, keepdims=True)
                    out.append(jnp.where(lane == j, r, accs[b]))
                return tuple(out)
            accs = (z, z) if "qabs" in dis else jax.lax.fori_loop(0, cpc, body, tuple(qabs_scr[b, cc] for b in range(NB)), unroll=unroll)
            for b in range(NB):
                qabs_scr[b, cc] = accs[b]

        def phase_b(t):
            j = t // NB
            b = t % NB

            @pl.when(b == 0)
            def _():
                base = pl.multiple_of(j * bchunk, bchunk)
                wait_all(ckv_v.at[:, pl.ds(base, bchunk)], SEM_CKV + j)
            if "b" in dis:
                return
            c = ckv_v[b, pl.ds(pl.multiple_of(j * bchunk, bchunk), bchunk), :]
            qabs = jnp.concatenate([qabs_scr[b, cc] for cc in range(DC // 128)], axis=1).astype(BF16)
            s = jax.lax.dot_general(qabs, c, (((1,), (1,)), ((), ())), preferred_element_type=F32) * (DH ** -0.5)
            m_prev = m_scr[b]
            m_new = jnp.maximum(m_prev, jnp.max(s, axis=1, keepdims=True))
            alpha = jnp.exp(m_prev - m_new)
            p = jnp.exp(s - m_new[:, 0:1])
            l_scr[b] = alpha * l_scr[b] + jnp.sum(p, axis=1, keepdims=True)
            m_scr[b] = m_new
            pv = jnp.dot(p.astype(BF16), c, preferred_element_type=F32)
            for cc in range(DC // 128):
                pc_scr[b, cc] = alpha * pc_scr[b, cc] + pv[:, cc * 128:(cc + 1) * 128]

        def phase_ctx(t):
            cc = t // (128 // cpc)
            j0 = (t % (128 // cpc)) * cpc

            @pl.when(t == 0)
            def _():
                wait_all(wuv_v, SEM_WUV)
            if "ctx" in dis:
                return
            pcs = [pc_scr[b, cc] / l_scr[b] for b in range(NB)]

            def body(jj, accs):
                j = j0 + jj
                w = wuv_v[cc * 128 + j].astype(F32)
                out = []
                for b in range(NB):
                    col = jnp.sum(jnp.where(lane == j, pcs[b], 0.0), axis=1, keepdims=True)
                    out.append(accs[b] + col * w)
                return tuple(out)
            accs = jax.lax.fori_loop(0, cpc, body, tuple(ctx_scr[b] for b in range(NB)), unroll=unroll)
            for b in range(NB):
                ctx_scr[b] = accs[b]

        def in_range(i, lo, n):
            return jnp.logical_and(i >= lo, i < lo + n)

        def head(i, c):
            slot = i % R

            @pl.when(i + LA < NHEAD)
            def _():
                start_head(i + LA, (i + LA) % R)

            for ci in range(min(LA, nch)):
                pl.when(i == NHEAD - LA + ci)(functools.partial(start_wo, ci))

            def pieces():
                @pl.when(in_range(i, i_qb, 2))
                def _():
                    phase_qb(i - i_qb)

                @pl.when(in_range(i, i_qabs, ncp))
                def _():
                    phase_qabs(i - i_qabs)

                @pl.when(in_range(i, i_b, NB * nbj))
                def _():
                    phase_b(i - i_b)

                @pl.when(in_range(i, i_ctx, ncp))
                def _():
                    phase_ctx(i - i_ctx)

            def extra_dma():
                pl.when(i == i_wu)(functools.partial(start_wu, 0))
                pl.when(i == i_wu + 1)(functools.partial(start_wu, 1))

                @pl.when(in_range(i, i_ckv, nbj))
                def _():
                    start_ckv(i - i_ckv)

            if piece_first:
                extra_dma()
                pieces()

            wait_all(kbuf.at[slot], SEM_K + slot)
            wait_all(vbuf.at[slot], SEM_V + slot)
            if "head" in dis:
                oa_scr[i] = qa_scr[i]
            else:
                q = qa_scr[i].astype(BF16)
                s = jax.lax.dot_general(q, kbuf[slot], (((1,), (1,)), ((), ())), preferred_element_type=F32) * (DH ** -0.5)
                m = jnp.max(s, axis=1, keepdims=True)
                p = jnp.exp(s - m)
                l = jnp.sum(p, axis=1, keepdims=True)
                oa_scr[i] = jnp.dot(p.astype(BF16), vbuf[slot], preferred_element_type=F32) / l

            if not piece_first:
                extra_dma()
                pieces()
            return c
        jax.lax.fori_loop(0, NHEAD, head, 0)

        for ci in range(min(LA, nch), nch):
            start_wo(ci)
        acc_a = jnp.zeros((16, DM), F32)
        acc_b = jnp.zeros((16, DM), F32)
        ctx = [ctx_scr[b] for b in range(NB)]
        for ci, (h0, nh) in enumerate(wo_chunks):
            la = jnp.concatenate([jnp.concatenate([oa_scr[b * NH + h] for b in range(NB)], axis=0) for h in range(h0, h0 + nh)], axis=1).astype(BF16)
            lb = jnp.concatenate([jnp.concatenate([jnp.broadcast_to(ctx[b][h:h + 1, :], (8, DH)) for b in range(NB)], axis=0) for h in range(h0, h0 + nh)], axis=1).astype(BF16)
            wait_all(wo_v.at[pl.ds(h0 * 128, nh * 128)], SEM_WO + ci)
            acc_a = acc_a + jnp.dot(la, wo_v[h0 * 128:(h0 + nh) * 128, :], preferred_element_type=F32)
            wait_all(wob_v.at[pl.ds(h0, nh)], SEM_WO + nch + ci)
            acc_b = acc_b + jnp.dot(lb, wob_v[h0:h0 + nh].reshape(nh * 128, DM), preferred_element_type=F32)
        ra = jnp.concatenate([acc_a[b * 8:b * 8 + 1, :] for b in range(NB)], axis=0)
        rb = jnp.concatenate([acc_b[b * 8:b * 8 + 1, :] for b in range(NB)], axis=0)
        o_ref[...] = jnp.concatenate([ra, rb], axis=1).astype(o_ref.dtype)

    def fn(A_x, A_k_cache, A_v_cache, A_wq, A_wo, B_x, B_c_kv, B_w_q, B_w_uk, B_w_uv, B_w_o):
        hbm = pl.BlockSpec(memory_space=pltpu.HBM)
        vm = pl.BlockSpec(memory_space=pltpu.VMEM)
        return pl.pallas_call(
            kernel,
            out_shape=jax.ShapeDtypeStruct((NB, 2 * DM), BF16),
            in_specs=[hbm] * 11,
            out_specs=vm,
            scratch_shapes=[
                pltpu.VMEM((R, S, DH), BF16), pltpu.VMEM((R, S, DH), BF16),
                pltpu.VMEM((DM, NH * DH), BF16), pltpu.VMEM((DM, NH, DH), BF16),
                pltpu.VMEM((DC, NH, DH), BF16), pltpu.VMEM((DC, NH, DH), BF16),
                pltpu.VMEM((NB, S, DC), BF16),
                pltpu.VMEM((NH * DH, DM), BF16), pltpu.VMEM((NH, DH, DM), BF16),
                pltpu.VMEM((NB, DM), BF16), pltpu.VMEM((NB, DM), BF16),
                pltpu.VMEM((8, DM), F32), pltpu.SMEM((8, DM), F32),
                pltpu.VMEM((NHEAD, 8, DH), F32), pltpu.VMEM((NHEAD, 8, DH), F32),
                pltpu.VMEM((NB, NH, DH), F32), pltpu.VMEM((NB, DC // 128, NH, DH), F32),
                pltpu.VMEM((NB, NH, DH), F32), pltpu.VMEM((NB, NH, DH), F32),
                pltpu.VMEM((NB, DC // 128, NH, DH), F32), pltpu.VMEM((NB, NH, DH), F32),
                pltpu.SemaphoreType.DMA((NSEM,)),
            ],
            compiler_params=pltpu.CompilerParams(vmem_limit_bytes=100 * 1024 * 1024, disable_bounds_checks=nbc),
        )(A_x.reshape(NB, DM), B_x.reshape(NB, DM), A_k_cache, A_v_cache, A_wq, A_wo, B_c_kv, B_w_q, B_w_uk, B_w_uv, B_w_o).reshape(NB, 1, 2 * DM)
    return fn


_FN = make_kernel()


@jax.jit
def pallas_concat_heads__gqa_block_cached__compressed_kv_cla__decode_kernel(
    A_x, A_k_cache, A_v_cache, A_wq, A_wo, B_x, B_c_kv, B_w_q, B_w_uk, B_w_uv, B_w_o,
):
    return _FN(A_x, A_k_cache, A_v_cache, A_wq, A_wo, B_x, B_c_kv, B_w_q, B_w_uk, B_w_uv, B_w_o)
```

```python
import contextlib
import functools
import jax
import jax.numpy as jnp
from jax.experimental import pallas as pl
from jax.experimental.pallas import tpu as pltpu

F32, BF16 = jnp.float32, jnp.bfloat16
NB, NH, S, DH, DM, DC = 2, 32, 8192, 128, 512, 512
NHEAD = NB * NH


def _pieces(total, step, start=0):
    out, o = [], 0
    while o < total:
        r = min(step, total - o)
        out.append((start + o, r))
        o += r
    return out


def _far(total, r, span):
    out, base = [], 0
    while base < total:
        blk = min(2 * span, total - base)
        s1 = span if blk == 2 * span else (blk + 1) // 2
        s2 = blk - s1
        p1, p2 = _pieces(s1, r), _pieces(s2, r)
        for t in range(max(len(p1), len(p2))):
            if t < len(p1):
                out.append((base + p1[t][0], p1[t][1], 0))
            if t < len(p2):
                out.append((base + s1 + p2[t][0], p2[t][1], 1))
        base += blk
    return out


def _kv_schedule(mode, rows, span):
    pcs = _pieces(S, rows)
    if mode == "kv":
        return [e for (o, r) in pcs for e in (("k", o, r, 0), ("v", o, r, 1))]
    if mode == "swap":
        return [e for t, (o, r) in enumerate(pcs) for e in (("k", o, r, t % 2), ("v", o, r, 1 - t % 2))]
    f = _far(S, rows, span)
    out = []
    for t in range(0, len(f), 2):
        p = (t // 2) % 2
        if mode == "quad":
            out += [("k",) + f[t], ("k",) + f[t + 1], ("v",) + f[t], ("v",) + f[t + 1]]
        elif mode == "quad2":
            out += [("k",) + f[t], ("v",) + f[t + 1], ("v",) + f[t], ("k",) + f[t + 1]]
        elif mode == "quad3":
            out += [("k", f[t][0], f[t][1], p), ("v", f[t][0], f[t][1], 1 - p),
                    ("k", f[t + 1][0], f[t + 1][1], 1 - p), ("v", f[t + 1][0], f[t + 1][1], p)]
        elif mode == "quad4":
            out += [("k", f[t][0], f[t][1], p), ("k", f[t + 1][0], f[t + 1][1], 1 - p),
                    ("v", f[t][0], f[t][1], 1 - p), ("v", f[t + 1][0], f[t + 1][1], p)]
    return out


def make_kernel(dis=(), kv_mode="quad4", kv_span=4096, kv_rows=192, slabs=6, ckv_rows=48, wo_rows=48, bchunk=2048,
                i_wu=0, i_ckv=2, i_wob=6, i_qb=0, i_qabs=3, i_b=12, i_ctx=21, i_bproj=30,
                wo_chunks=((0, 16), (16, 8), (24, 4), (28, 4)), unroll=8, nbc=False, cpc=64, R=3,
                ex_swap=True, scopes=False, wob_late=False, wo_far=False, nsc=False, sdb=False, region_proj=False):
    kv_sched = _kv_schedule(kv_mode, kv_rows, kv_span)
    nch = len(wo_chunks)
    nbj = S // bchunk
    ncp = DC // cpc
    SEM_A = 0
    SEM_B = 1
    SEM_WQ = 2
    SEM_WU = 3
    SEM_WO = 4
    SEM_KV = SEM_WO + nch
    NSEM = SEM_KV + R
    SEM_AX, SEM_BX, SEM_X, SEM_WOB, SEM_CKV = SEM_A, SEM_B, SEM_B, SEM_A, SEM_B
    LA = R - 1

    def sc(name):
        return jax.named_scope(name) if scopes else contextlib.nullcontext()

    def kernel(ax_hbm, bx_hbm, k_hbm, v_hbm, wq_hbm, wo_hbm, ckv_hbm, wqb_hbm, wuk_hbm, wuv_hbm, wob_hbm,
               o_ref,
               kbuf, vbuf, wq_v, wqb_v, wuk_v, wuv_v, ckv_v, wo_v, wob_v,
               ax_v, bx_v, xb_v, xb_s, qa_scr, oa_scr, qb_scr, qabs_scr, m_scr, l_scr, pc_scr, ctx_scr, ob_scr, oaa_scr, sems):

        def copy(src, dst, sem):
            return pltpu.make_async_copy(src, dst, sems.at[sem])

        def wait_all(buf, sem):
            pltpu.make_async_copy(buf, buf, sems.at[sem]).wait()

        def issue_pairs(a, b):
            for t in range(max(len(a), len(b))):
                p = t % 2 if ex_swap else 0
                if t < len(a):
                    copy(*a[t]).start(priority=p)
                if t < len(b):
                    copy(*b[t]).start(priority=1 - p)

        def start_head(i, slot):
            b = i // NH
            h = i % NH
            for (w, o, r, p) in kv_sched:
                if w == "k":
                    copy(k_hbm.at[b, h, pl.ds(o, r)], kbuf.at[slot, pl.ds(o, r)], SEM_KV + slot).start(priority=p)
                else:
                    copy(v_hbm.at[b, h, pl.ds(o, r)], vbuf.at[slot, pl.ds(o, r)], SEM_KV + slot).start(priority=p)

        def start_wq_pair():
            a = [(wq_hbm.at[pl.ds(r, 16), pl.ds(c, n)], wq_v.at[pl.ds(r, 16), pl.ds(c, n)], SEM_WQ)
                 for r in range(0, DM, 16) for (c, n) in ((0, 1536), (1536, 1536), (3072, 1024))]
            b = [(wqb_hbm.at[pl.ds(o, n)], wqb_v.at[pl.ds(o, n)], SEM_WQ) for (o, n) in _pieces(DM, slabs)]
            issue_pairs(a, b)

        def start_wu(half):
            pcs = _pieces(DM, slabs)
            hh = (len(pcs) + 1) // 2
            pcs = pcs[:hh] if half == 0 else pcs[hh:]
            issue_pairs([(wuk_hbm.at[pl.ds(o, n)], wuk_v.at[pl.ds(o, n)], SEM_WU) for (o, n) in pcs],
                        [(wuv_hbm.at[pl.ds(o, n)], wuv_v.at[pl.ds(o, n)], SEM_WU) for (o, n) in pcs])

        def start_ckv(j):
            base = pl.multiple_of(j * bchunk, bchunk)
            pcs = _pieces(bchunk, ckv_rows)
            issue_pairs([(ckv_hbm.at[0, pl.ds(base + o, r)], ckv_v.at[0, pl.ds(base + o, r)], SEM_CKV) for (o, r) in pcs],
                        [(ckv_hbm.at[1, pl.ds(base + o, r)], ckv_v.at[1, pl.ds(base + o, r)], SEM_CKV) for (o, r) in pcs])

        def wob_list(h0, nh):
            return [(wob_hbm.at[h, pl.ds(o, r)], wob_v.at[h, pl.ds(o, r)], SEM_WOB) for h in range(h0, h0 + nh) for (o, r) in _pieces(128, wo_rows)]

        def start_wob():
            issue_pairs(wob_list(0, NH // 2), wob_list(NH // 2, NH // 2))

        def start_wo(ci):
            h0, nh = wo_chunks[ci]
            pcs = _pieces(nh * 128, wo_rows, h0 * 128)
            lst = [(wo_hbm.at[pl.ds(o, r)], wo_v.at[pl.ds(o, r)], SEM_WO + ci) for (o, r) in pcs]
            if wo_far:
                hh = (len(lst) + 1) // 2
                issue_pairs(lst[:hh], lst[hh:])
            else:
                issue_pairs(lst[0::2], lst[1::2])

        ax_copy = copy(ax_hbm, ax_v, SEM_AX)
        bx_copy = copy(bx_hbm, bx_v, SEM_BX)
        ax_copy.start(priority=0)
        bx_copy.start(priority=1)
        with sc("s_pro_wq"):
            start_wq_pair()
        with sc("s_pro_heads"):
            for i0 in range(LA):
                start_head(i0, i0)

        ax_copy.wait()
        bx_copy.wait()
        axf = ax_v[...].astype(F32)
        xa = jnp.concatenate([jnp.broadcast_to(axf[b:b + 1, :], (8, DM)) for b in range(NB)], axis=0).astype(BF16)
        xb_v[...] = jnp.concatenate([bx_v[...].astype(F32), jnp.zeros((8 - NB, DM), F32)], axis=0)
        xcopy = copy(xb_v, xb_s, SEM_X)
        xcopy.start()

        z = jnp.zeros((NH, DH), F32)
        for b in range(NB):
            qb_scr[b] = z
            ctx_scr[b] = z
            m_scr[b] = jnp.full((NH, DH), -jnp.inf, F32)
            l_scr[b] = z
            for cc in range(DC // 128):
                pc_scr[b, cc] = z
                qabs_scr[b, cc] = z

        with sc("s_qa"):
            wait_all(wq_v, SEM_WQ)
            wait_all(wqb_v, SEM_WQ)
            qa = jnp.dot(xa, wq_v[...], preferred_element_type=F32)
            for b in range(NB):
                for h in range(NH):
                    qa_scr[b * NH + h] = qa[b * 8:(b + 1) * 8, h * DH:(h + 1) * DH]

        lane = jax.lax.broadcasted_iota(jnp.int32, (NH, DH), 1)

        def phase_qb(part):
            @pl.when(part == 0)
            def _():
                xcopy.wait()
            if "qb" in dis:
                return
            m0 = part * (DM // 2)

            def body(t, accs):
                m = m0 + t
                w = wqb_v[m].astype(F32)
                return tuple(accs[b] + w * xb_s[b, m] for b in range(NB))
            accs = jax.lax.fori_loop(0, DM // 2, body, tuple(qb_scr[b] for b in range(NB)), unroll=unroll)
            for b in range(NB):
                qb_scr[b] = accs[b]

        def phase_qabs(t):
            cc = t // (128 // cpc)
            j0 = (t % (128 // cpc)) * cpc

            @pl.when(t == 0)
            def _():
                wait_all(wuk_v, SEM_WU)
                wait_all(wuv_v, SEM_WU)
            if "qabs" in dis:
                return
            q = [qb_scr[b] for b in range(NB)]

            def body(jj, accs):
                j = j0 + jj
                w = wuk_v[cc * 128 + j].astype(F32)
                out = []
                for b in range(NB):
                    r = jnp.sum(w * q[b], axis=1, keepdims=True)
                    out.append(jnp.where(lane == j, r, accs[b]))
                return tuple(out)
            accs = jax.lax.fori_loop(0, cpc, body, tuple(qabs_scr[b, cc] for b in range(NB)), unroll=unroll)
            for b in range(NB):
                qabs_scr[b, cc] = accs[b]

        def phase_b(t):
            j = t // NB
            b = t % NB

            @pl.when(t == 0)
            def _():
                wait_all(ckv_v, SEM_CKV)
            if "b" in dis:
                return
            c = ckv_v[b, pl.ds(pl.multiple_of(j * bchunk, bchunk), bchunk), :]
            qabs = jnp.concatenate([qabs_scr[b, cc] for cc in range(DC // 128)], axis=1).astype(BF16)
            s = jax.lax.dot_general(qabs, c, (((1,), (1,)), ((), ())), preferred_element_type=F32) * (DH ** -0.5)
            m_prev = m_scr[b]
            m_new = jnp.maximum(m_prev, jnp.max(s, axis=1, keepdims=True))
            alpha = jnp.exp(m_prev - m_new)
            p = jnp.exp(s - m_new[:, 0:1])
            l_scr[b] = alpha * l_scr[b] + jnp.sum(p, axis=1, keepdims=True)
            m_scr[b] = m_new
            pv = jnp.dot(p.astype(BF16), c, preferred_element_type=F32)
            for cc in range(DC // 128):
                pc_scr[b, cc] = alpha * pc_scr[b, cc] + pv[:, cc * 128:(cc + 1) * 128]

        def phase_ctx(t):
            cc = t // (128 // cpc)
            j0 = (t % (128 // cpc)) * cpc

            if "ctx" in dis:
                return
            pcs = [pc_scr[b, cc] / l_scr[b] for b in range(NB)]

            def body(jj, accs):
                j = j0 + jj
                w = wuv_v[cc * 128 + j].astype(F32)
                out = []
                for b in range(NB):
                    col = jnp.sum(jnp.where(lane == j, pcs[b], 0.0), axis=1, keepdims=True)
                    out.append(accs[b] + col * w)
                return tuple(out)
            accs = jax.lax.fori_loop(0, cpc, body, tuple(ctx_scr[b] for b in range(NB)), unroll=unroll)
            for b in range(NB):
                ctx_scr[b] = accs[b]

        def phase_bproj():
            wait_all(wob_v, SEM_WOB)
            ctx = [ctx_scr[b] for b in range(NB)]
            lb = jnp.concatenate([jnp.concatenate([jnp.broadcast_to(ctx[b][h:h + 1, :], (8, DH)) for b in range(NB)], axis=0) for h in range(NH)], axis=1).astype(BF16)
            ob_scr[...] = jnp.dot(lb, wob_v[...].reshape(NH * DH, DM), preferred_element_type=F32)

        def in_range(i, lo, n):
            return jnp.logical_and(i >= lo, i < lo + n)

        def head(i, c):
            slot = i % R
            with sc("s_start_head"):
                @pl.when(i + LA < NHEAD)
                def _():
                    start_head(i + LA, (i + LA) % R)

            for ci in range(min(LA, nch)):
                pl.when(i == NHEAD - LA + ci)(functools.partial(start_wo, ci))

            def attend():
                wait_all(kbuf.at[slot], SEM_KV + slot)
                wait_all(vbuf.at[slot], SEM_KV + slot)
                if "head" in dis:
                    oa_scr[i] = qa_scr[i]
                    return
                q = qa_scr[i].astype(BF16)
                s = jax.lax.dot_general(q, kbuf[slot], (((1,), (1,)), ((), ())), preferred_element_type=F32) * (DH ** -0.5)
                m = jnp.max(s, axis=1, keepdims=True)
                p = jnp.exp(s - m)
                l = jnp.sum(p, axis=1, keepdims=True)
                oa_scr[i] = jnp.dot(p.astype(BF16), vbuf[slot], preferred_element_type=F32) / l
            if scopes:
                with sc("s_head"):
                    pl.when(i >= 0)(attend)
            else:
                attend()

            with sc("s_extra_dma"):
                pl.when(i == i_wu)(functools.partial(start_wu, 0))
                pl.when(i == i_wu + 1)(functools.partial(start_wu, 1))

                @pl.when(in_range(i, i_ckv, nbj))
                def _():
                    start_ckv(i - i_ckv)

                pl.when(i == i_wob)(start_wob)

            with sc("s_pieces"):
                @pl.when(in_range(i, i_qb, 2))
                def _():
                    phase_qb(i - i_qb)

                @pl.when(in_range(i, i_qabs, ncp))
                def _():
                    phase_qabs(i - i_qabs)

                @pl.when(in_range(i, i_b, NB * nbj))
                def _():
                    phase_b(i - i_b)

                @pl.when(in_range(i, i_ctx, ncp))
                def _():
                    phase_ctx(i - i_ctx)

                pl.when(i == i_bproj)(phase_bproj)
            return c
        jax.lax.fori_loop(0, NHEAD, head, 0)

        with sc("s_start_wo_rest"):
            for ci in range(min(LA, nch), nch):
                start_wo(ci)
        always = xb_s[2, 0] == 0.0
        for ci, (h0, nh) in enumerate(wo_chunks):
            def proj(ci=ci, h0=h0, nh=nh):
                wait_all(wo_v.at[pl.ds(h0 * 128, nh * 128)], SEM_WO + ci)
                la = jnp.concatenate([jnp.concatenate([oa_scr[b * NH + h] for b in range(NB)], axis=0) for h in range(h0, h0 + nh)], axis=1).astype(BF16)
                d = jnp.dot(la, wo_v[h0 * 128:(h0 + nh) * 128, :], preferred_element_type=F32)
                oaa_scr[...] = d if ci == 0 else oaa_scr[...] + d
            with sc(f"s_projA{ci}"):
                if region_proj:
                    pl.when(always)(proj)
                else:
                    proj()
        acc_a = oaa_scr[...]
        with sc("s_final"):
            acc_b = ob_scr[...]
            ra = jnp.concatenate([acc_a[b * 8:b * 8 + 1, :] for b in range(NB)], axis=0)
            rb = jnp.concatenate([acc_b[b * 8:b * 8 + 1, :] for b in range(NB)], axis=0)
            o_ref[...] = jnp.concatenate([ra, rb], axis=1).astype(o_ref.dtype)

    def fn(A_x, A_k_cache, A_v_cache, A_wq, A_wo, B_x, B_c_kv, B_w_q, B_w_uk, B_w_uv, B_w_o):
        hbm = pl.BlockSpec(memory_space=pltpu.HBM)
        vm = pl.BlockSpec(memory_space=pltpu.VMEM)
        return pl.pallas_call(
            kernel,
            out_shape=jax.ShapeDtypeStruct((NB, 2 * DM), BF16),
            in_specs=[hbm] * 11,
            out_specs=vm,
            scratch_shapes=[
                pltpu.VMEM((R, S, DH), BF16), pltpu.VMEM((R, S, DH), BF16),
                pltpu.VMEM((DM, NH * DH), BF16), pltpu.VMEM((DM, NH, DH), BF16),
                pltpu.VMEM((DC, NH, DH), BF16), pltpu.VMEM((DC, NH, DH), BF16),
                pltpu.VMEM((NB, S, DC), BF16),
                pltpu.VMEM((NH * DH, DM), BF16), pltpu.VMEM((NH, DH, DM), BF16),
                pltpu.VMEM((NB, DM), BF16), pltpu.VMEM((NB, DM), BF16),
                pltpu.VMEM((8, DM), F32), pltpu.SMEM((8, DM), F32),
                pltpu.VMEM((NHEAD, 8, DH), F32), pltpu.VMEM((NHEAD, 8, DH), F32),
                pltpu.VMEM((NB, NH, DH), F32), pltpu.VMEM((NB, DC // 128, NH, DH), F32),
                pltpu.VMEM((NB, NH, DH), F32), pltpu.VMEM((NB, NH, DH), F32),
                pltpu.VMEM((NB, DC // 128, NH, DH), F32), pltpu.VMEM((NB, NH, DH), F32),
                pltpu.VMEM((16, DM), F32), pltpu.VMEM((16, DM), F32),
                pltpu.SemaphoreType.DMA((NSEM,)),
            ],
            compiler_params=pltpu.CompilerParams(vmem_limit_bytes=100 * 1024 * 1024, disable_bounds_checks=nbc, disable_semaphore_checks=nsc, skip_device_barrier=sdb),
        )(A_x.reshape(NB, DM), B_x.reshape(NB, DM), A_k_cache, A_v_cache, A_wq, A_wo, B_c_kv, B_w_q, B_w_uk, B_w_uv, B_w_o).reshape(NB, 1, 2 * DM)
    return fn


_FN = make_kernel()


@jax.jit
def pallas_concat_heads__gqa_block_cached__compressed_kv_cla__decode_kernel(
    A_x, A_k_cache, A_v_cache, A_wq, A_wo, B_x, B_c_kv, B_w_q, B_w_uk, B_w_uv, B_w_o,
):
    return _FN(A_x, A_k_cache, A_v_cache, A_wq, A_wo, B_x, B_c_kv, B_w_q, B_w_uk, B_w_uv, B_w_o)
```

```python
import functools

import jax
import jax.numpy as jnp
from jax.experimental import pallas as pl
from jax.experimental.pallas import tpu as pltpu

F32, BF16 = jnp.float32, jnp.bfloat16
NB, NH, S, DH, DM, DC = 2, 32, 8192, 128, 512, 512
NHEAD = NB * NH
NCC = DC // 128

R = 3
LA = R - 1
KV_ROWS = 160
SLABS = 6
WIDE_ROWS = 48
BCHUNK = 2048
NBJ = S // BCHUNK
CPC = 64
NCP = DC // CPC
WO_CHUNKS = ((0, 16), (16, 8), (24, 4), (28, 4))
NCH = len(WO_CHUNKS)

I_WU, I_CKV, I_WOB = 0, 2, 6
I_QB, I_QABS, I_B, I_CTX, I_BPROJ = 0, 3, 12, 21, 30

SEM_A = 0
SEM_B = 1
SEM_WQ = 2
SEM_WU = 3
SEM_WO = 4
SEM_KV = SEM_WO + NCH
NSEM = SEM_KV + R


def _pieces(total, step, start=0):
    return [(start + o, min(step, total - o)) for o in range(0, total, step)]


def _kv_schedule():
    lo, hi = _pieces(S // 2, KV_ROWS), _pieces(S // 2, KV_ROWS, S // 2)
    out = []
    for t, (a, b) in enumerate(zip(lo, hi)):
        p = t % 2
        out += [("k", *a, p), ("k", *b, 1 - p), ("v", *a, p), ("v", *b, 1 - p)]
    return out


KV_SCHEDULE = _kv_schedule()


def _kernel(ax_hbm, bx_hbm, k_hbm, v_hbm, wq_hbm, wo_hbm, ckv_hbm, wqb_hbm, wuk_hbm, wuv_hbm, wob_hbm,
            o_ref,
            kbuf, vbuf, wq_v, wqb_v, wuk_v, wuv_v, ckv_v, wo_v, wob_v, ax_v, bx_v,
            xb_scr, qa_scr, oa_scr, qb_scr, qabs_scr, m_scr, l_scr, pc_scr, ctx_scr, outa_scr, outb_scr,
            sems):

    def copy(src, dst, sem):
        return pltpu.make_async_copy(src, dst, sems.at[sem])

    def wait_all(buf, sem):
        pltpu.make_async_copy(buf, buf, sems.at[sem]).wait()

    def issue_pairs(a, b):
        for t in range(max(len(a), len(b))):
            if t < len(a):
                copy(*a[t]).start(priority=t % 2)
            if t < len(b):
                copy(*b[t]).start(priority=1 - t % 2)

    def start_head(i, slot):
        b, h = i // NH, i % NH
        for name, o, r, p in KV_SCHEDULE:
            src, dst = (k_hbm, kbuf) if name == "k" else (v_hbm, vbuf)
            copy(src.at[b, h, pl.ds(o, r)], dst.at[slot, pl.ds(o, r)], SEM_KV + slot).start(priority=p)

    def start_wq():
        a = [(wq_hbm.at[pl.ds(r, 16), pl.ds(c, n)], wq_v.at[pl.ds(r, 16), pl.ds(c, n)], SEM_WQ)
             for r in range(0, DM, 16) for c, n in _pieces(NH * DH, 1536)]
        b = [(wqb_hbm.at[pl.ds(o, n)], wqb_v.at[pl.ds(o, n)], SEM_WQ) for o, n in _pieces(DM, SLABS)]
        issue_pairs(a, b)

    def start_wu(half):
        pcs = _pieces(DC // 2, SLABS, half * (DC // 2))
        issue_pairs([(wuk_hbm.at[pl.ds(o, n)], wuk_v.at[pl.ds(o, n)], SEM_WU) for o, n in pcs],
                    [(wuv_hbm.at[pl.ds(o, n)], wuv_v.at[pl.ds(o, n)], SEM_WU) for o, n in pcs])

    def start_ckv(j):
        base = pl.multiple_of(j * BCHUNK, BCHUNK)
        pcs = _pieces(BCHUNK, WIDE_ROWS)
        issue_pairs(*[[(ckv_hbm.at[b, pl.ds(base + o, r)], ckv_v.at[b, pl.ds(base + o, r)], SEM_B) for o, r in pcs]
                      for b in range(NB)])

    def start_wob():
        issue_pairs(*[[(wob_hbm.at[h, pl.ds(o, r)], wob_v.at[h, pl.ds(o, r)], SEM_A)
                       for h in range(h0, h0 + NH // 2) for o, r in _pieces(DH, WIDE_ROWS)]
                      for h0 in (0, NH // 2)])

    def start_wo(ci):
        h0, nh = WO_CHUNKS[ci]
        lst = [(wo_hbm.at[pl.ds(o, r)], wo_v.at[pl.ds(o, r)], SEM_WO + ci)
               for o, r in _pieces(nh * DH, WIDE_ROWS, h0 * DH)]
        issue_pairs(lst[0::2], lst[1::2])

    ax_copy, bx_copy = copy(ax_hbm, ax_v, SEM_A), copy(bx_hbm, bx_v, SEM_B)
    ax_copy.start(priority=0)
    bx_copy.start(priority=1)
    start_wq()
    for i0 in range(LA):
        start_head(i0, i0)

    ax_copy.wait()
    bx_copy.wait()
    ax, bx = ax_v[...].astype(F32), bx_v[...].astype(F32)
    xa = jnp.concatenate([jnp.broadcast_to(ax[b:b + 1, :], (8, DM)) for b in range(NB)], axis=0).astype(BF16)
    zero = jnp.zeros((NH, DH), F32)
    for b in range(NB):
        for cc in range(DM // 128):
            xb_scr[b, cc] = jnp.broadcast_to(bx[b:b + 1, cc * 128:(cc + 1) * 128], (8, 128))
        for cc in range(NCC):
            qabs_scr[b, cc] = zero
            pc_scr[b, cc] = zero
        qb_scr[b] = zero
        ctx_scr[b] = zero
        l_scr[b] = zero
        m_scr[b] = jnp.full((NH, DH), -jnp.inf, F32)

    wait_all(wq_v, SEM_WQ)
    wait_all(wqb_v, SEM_WQ)
    qa = jnp.dot(xa, wq_v[...], preferred_element_type=F32)
    for b in range(NB):
        for h in range(NH):
            qa_scr[b * NH + h] = qa[b * 8:(b + 1) * 8, h * DH:(h + 1) * DH]

    lane = jax.lax.broadcasted_iota(jnp.int32, (NH, DH), 1)
    lane8 = jax.lax.broadcasted_iota(jnp.int32, (8, DH), 1)

    def part_qb(t):
        accs = tuple(qb_scr[b] for b in range(NB))
        for half in range(2):
            cc = t * 2 + half
            xs = [xb_scr[b, cc] for b in range(NB)]

            def body(j, accs):
                w = wqb_v[cc * 128 + j].astype(F32).reshape(NH // 8, 8, DH)
                out = []
                for b in range(NB):
                    xm = jnp.sum(jnp.where(lane8 == j, xs[b], 0.0), axis=1, keepdims=True)
                    out.append(accs[b] + (w * xm[None]).reshape(NH, DH))
                return tuple(out)
            accs = jax.lax.fori_loop(0, 128, body, accs, unroll=8)
        for b in range(NB):
            qb_scr[b] = accs[b]

    def part_qabs(t):
        cc, j0 = t // (128 // CPC), (t % (128 // CPC)) * CPC

        @pl.when(t == 0)
        def _():
            wait_all(wuk_v, SEM_WU)
            wait_all(wuv_v, SEM_WU)
        q = [qb_scr[b] for b in range(NB)]

        def body(jj, accs):
            j = j0 + jj
            w = wuk_v[cc * 128 + j].astype(F32)
            return tuple(jnp.where(lane == j, jnp.sum(w * q[b], axis=1, keepdims=True), accs[b])
                         for b in range(NB))
        accs = jax.lax.fori_loop(0, CPC, body, tuple(qabs_scr[b, cc] for b in range(NB)), unroll=8)
        for b in range(NB):
            qabs_scr[b, cc] = accs[b]

    def part_latent_attention(t):
        j, b = t // NB, t % NB

        @pl.when(t == 0)
        def _():
            wait_all(ckv_v, SEM_B)
        c = ckv_v[b, pl.ds(pl.multiple_of(j * BCHUNK, BCHUNK), BCHUNK), :]
        qabs = jnp.concatenate([qabs_scr[b, cc] for cc in range(NCC)], axis=1).astype(BF16)
        s = jax.lax.dot_general(qabs, c, (((1,), (1,)), ((), ())), preferred_element_type=F32) * (DH ** -0.5)
        m_prev = m_scr[b]
        m_new = jnp.maximum(m_prev, jnp.max(s, axis=1, keepdims=True))
        alpha = jnp.exp(m_prev - m_new)
        p = jnp.exp(s - m_new[:, 0:1])
        l_scr[b] = alpha * l_scr[b] + jnp.sum(p, axis=1, keepdims=True)
        m_scr[b] = m_new
        pv = jnp.dot(p.astype(BF16), c, preferred_element_type=F32)
        for cc in range(NCC):
            pc_scr[b, cc] = alpha * pc_scr[b, cc] + pv[:, cc * 128:(cc + 1) * 128]

    def part_ctx(t):
        cc, j0 = t // (128 // CPC), (t % (128 // CPC)) * CPC
        pcs = [pc_scr[b, cc] / l_scr[b] for b in range(NB)]

        def body(jj, accs):
            j = j0 + jj
            w = wuv_v[cc * 128 + j].astype(F32)
            return tuple(accs[b] + jnp.sum(jnp.where(lane == j, pcs[b], 0.0), axis=1, keepdims=True) * w
                         for b in range(NB))
        accs = jax.lax.fori_loop(0, CPC, body, tuple(ctx_scr[b] for b in range(NB)), unroll=8)
        for b in range(NB):
            ctx_scr[b] = accs[b]

    def part_out_b():
        wait_all(wob_v, SEM_A)
        ctx = [ctx_scr[b] for b in range(NB)]
        lhs = jnp.concatenate(
            [jnp.concatenate([jnp.broadcast_to(ctx[b][h:h + 1, :], (8, DH)) for b in range(NB)], axis=0)
             for h in range(NH)], axis=1).astype(BF16)
        outb_scr[...] = jnp.dot(lhs, wob_v[...].reshape(NH * DH, DM), preferred_element_type=F32)

    def in_range(i, lo, n):
        return jnp.logical_and(i >= lo, i < lo + n)

    def run_in_range(i, lo, n, fn):
        @pl.when(in_range(i, lo, n))
        def _():
            fn(i - lo)

    def head(i, carry):
        slot = i % R

        @pl.when(i + LA < NHEAD)
        def _():
            start_head(i + LA, (i + LA) % R)

        for ci in range(min(LA, NCH)):
            pl.when(i == NHEAD - LA + ci)(functools.partial(start_wo, ci))

        wait_all(kbuf.at[slot], SEM_KV + slot)
        wait_all(vbuf.at[slot], SEM_KV + slot)
        q = qa_scr[i].astype(BF16)
        s = jax.lax.dot_general(q, kbuf[slot], (((1,), (1,)), ((), ())), preferred_element_type=F32) * (DH ** -0.5)
        p = jnp.exp(s - jnp.max(s, axis=1, keepdims=True))
        l = jnp.sum(p, axis=1, keepdims=True)
        oa_scr[i] = jnp.dot(p.astype(BF16), vbuf[slot], preferred_element_type=F32) / l

        for half in range(2):
            pl.when(i == I_WU + half)(functools.partial(start_wu, half))
        run_in_range(i, I_CKV, NBJ, start_ckv)
        pl.when(i == I_WOB)(start_wob)

        run_in_range(i, I_QB, 2, part_qb)
        run_in_range(i, I_QABS, NCP, part_qabs)
        run_in_range(i, I_B, NB * NBJ, part_latent_attention)
        run_in_range(i, I_CTX, NCP, part_ctx)
        pl.when(i == I_BPROJ)(part_out_b)
        return carry

    jax.lax.fori_loop(0, NHEAD, head, 0)

    for ci in range(min(LA, NCH), NCH):
        start_wo(ci)
    for ci, (h0, nh) in enumerate(WO_CHUNKS):
        lhs = jnp.concatenate(
            [jnp.concatenate([oa_scr[b * NH + h] for b in range(NB)], axis=0) for h in range(h0, h0 + nh)],
            axis=1).astype(BF16)
        wait_all(wo_v.at[pl.ds(h0 * DH, nh * DH)], SEM_WO + ci)
        d = jnp.dot(lhs, wo_v[h0 * DH:(h0 + nh) * DH, :], preferred_element_type=F32)
        outa_scr[...] = d if ci == 0 else outa_scr[...] + d

    rows = [jnp.concatenate([outa_scr[b * 8:b * 8 + 1, :], outb_scr[b * 8:b * 8 + 1, :]], axis=1) for b in range(NB)]
    o_ref[...] = jnp.concatenate(rows, axis=0).astype(o_ref.dtype)


@jax.jit
def pallas_concat_heads__gqa_block_cached__compressed_kv_cla__decode_kernel(
    A_x: jax.Array,
    A_k_cache: jax.Array,
    A_v_cache: jax.Array,
    A_wq: jax.Array,
    A_wo: jax.Array,
    B_x: jax.Array,
    B_c_kv: jax.Array,
    B_w_q: jax.Array,
    B_w_uk: jax.Array,
    B_w_uv: jax.Array,
    B_w_o: jax.Array,
):
    out = pl.pallas_call(
        _kernel,
        out_shape=jax.ShapeDtypeStruct((NB, 2 * DM), BF16),
        in_specs=[pl.BlockSpec(memory_space=pltpu.HBM)] * 11,
        out_specs=pl.BlockSpec(memory_space=pltpu.VMEM),
        scratch_shapes=[
            pltpu.VMEM((R, S, DH), BF16),
            pltpu.VMEM((R, S, DH), BF16),
            pltpu.VMEM((DM, NH * DH), BF16),
            pltpu.VMEM((DM, NH, DH), BF16),
            pltpu.VMEM((DC, NH, DH), BF16),
            pltpu.VMEM((DC, NH, DH), BF16),
            pltpu.VMEM((NB, S, DC), BF16),
            pltpu.VMEM((NH * DH, DM), BF16),
            pltpu.VMEM((NH, DH, DM), BF16),
            pltpu.VMEM((NB, DM), BF16),
            pltpu.VMEM((NB, DM), BF16),
            pltpu.VMEM((NB, DM // 128, 8, 128), F32),
            pltpu.VMEM((NHEAD, 8, DH), F32),
            pltpu.VMEM((NHEAD, 8, DH), F32),
            pltpu.VMEM((NB, NH, DH), F32),
            pltpu.VMEM((NB, NCC, NH, DH), F32),
            pltpu.VMEM((NB, NH, DH), F32),
            pltpu.VMEM((NB, NH, DH), F32),
            pltpu.VMEM((NB, NCC, NH, DH), F32),
            pltpu.VMEM((NB, NH, DH), F32),
            pltpu.VMEM((16, DM), F32),
            pltpu.VMEM((16, DM), F32),
            pltpu.SemaphoreType.DMA((NSEM,)),
        ],
        compiler_params=pltpu.CompilerParams(vmem_limit_bytes=100 * 1024 * 1024),
    )(A_x.reshape(NB, DM), B_x.reshape(NB, DM), A_k_cache, A_v_cache, A_wq, A_wo,
      B_c_kv, B_w_q, B_w_uk, B_w_uv, B_w_o)
    return out.reshape(NB, 1, 2 * DM)
```
